```python
import os as _os
_os.environ.setdefault("JAX_PLATFORMS", "cpu")
import jax
import jax.numpy as jnp

def _softmax(x, axis=-1):
    return jax.nn.softmax(x, axis=axis)
def _gelu(x):
    return jax.nn.gelu(x, approximate=True)
def _silu(x):
    return jax.nn.silu(x)
def _sigmoid(x):
    return jax.nn.sigmoid(x)
def _layernorm(x, axis=-1, eps=1e-5):
    m = jnp.mean(x, axis=axis, keepdims=True)
    v = jnp.var(x, axis=axis, keepdims=True)
    return (x - m) / jnp.sqrt(v + eps)
def _scatter_add(tgt, idx, src, axis=0):
    return tgt.at[idx].add(src)
def _segment_sum(src, seg, n):
    return jax.ops.segment_sum(src, seg, n)
class _Rng:
    def __init__(self, key):
        self._k = key
    def _next(self):
        self._k, sub = jax.random.split(self._k)
        return sub
    def normal(self, shape):
        return jax.random.normal(self._next(), shape, dtype=jnp.bfloat16)
    def randint(self, lo, hi, shape):
        return jax.random.randint(self._next(), shape, lo, hi, dtype=jnp.int32)
    def uniform(self, shape, lo=0.0, hi=1.0):
        return jax.random.uniform(self._next(), shape, jnp.bfloat16, lo, hi)
    def permutation(self, n):
        return jax.random.permutation(self._next(), n)


kernel_name = 'gated_mix__gqa_block_cached__dense_activation_squared_relu__decode'

def setup_inputs():
    _rng = _Rng(jax.random.key(int.from_bytes(__import__("os").urandom(4), "little")))
    _w = (lambda a: (lambda t: t.astype(jnp.bfloat16) if jnp.issubdtype(t.dtype, jnp.floating) else t)(jnp.asarray(a)))
    def _A_setup():
        B, Sq, D = 4, 1, 512
        Hq, Hkv, Sk, Dh = 32, 8, 4096, 128
        assert Hq % Hkv == 0, (Hq, Hkv)
        return {
            "x": _w((lambda *s: _rng.normal(s) * 0.05)(B, Sq, D)),
            "k_cache": _w((lambda *s: _rng.normal(s) * 3.2)(B, Hkv, Sk, Dh)),
            "v_cache": _w((lambda *s: _rng.normal(s) * 1.6)(B, Hkv, Sk, Dh)),
            "wq": _w((lambda *s: _rng.normal(s) * 3.2)(D, Hq * Dh) * (D ** -0.5)),
            "wo": _w((lambda *s: _rng.normal(s) * 1.6)(Hq * Dh, D) * ((Hq * Dh) ** -0.5)),
        }
    _A_in = _A_setup()

    def _B_setup():
        B, S, D, F = 4, 1, 512, 1792
        return {
            "x": _w((lambda *s: _rng.normal(s) * 0.05)(B, S, D)),
            "w1": _w((lambda *s: _rng.normal(s) * 0.1)(D, F)),
            "b1": _w((lambda *s: _rng.normal(s) * 0.05)(F)),
            "w2": _w((lambda *s: _rng.normal(s) * 0.05)(F, D)),
            "b2": _w((lambda *s: _rng.normal(s) * 0.05)(D)),
        }
    _B_in = _B_setup()

    return {
        "A_x": _A_in["x"],
        "A_k_cache": _A_in["k_cache"],
        "A_v_cache": _A_in["v_cache"],
        "A_wq": _A_in["wq"],
        "A_wo": _A_in["wo"],
        "B_x": _B_in["x"],
        "B_w1": _B_in["w1"],
        "B_b1": _B_in["b1"],
        "B_w2": _B_in["w2"],
        "B_b2": _B_in["b2"],
        "gate_w": _w((lambda *s: _rng.normal(s) * 0.05)(512) * 16.0),
    }

def reference(A_x, A_k_cache, A_v_cache, A_wq, A_wo, B_x, B_w1, B_b1, B_w2, B_b2, gate_w):
    def _A_ref(x, k_cache, v_cache, wq, wo):
        B, Sq, D = x.shape
        Hq, Dh = 32, 128
        Hkv = k_cache.shape[1]
        rep = Hq // Hkv
        q = (lambda x, *d: x.transpose(*d))((x @ wq).reshape(B, Sq, Hq, Dh), 0, 2, 1, 3)
        k = jnp.repeat(k_cache, rep, axis=1)
        v = jnp.repeat(v_cache, rep, axis=1)
        scores = jnp.einsum("bhqd,bhkd->bhqk", q, k) * (Dh ** -0.5)
        p = _softmax(scores, axis=-1)
        o = jnp.einsum("bhqk,bhkd->bhqd", p, v)
        return (lambda x, *d: x.transpose(*d))(o, 0, 2, 1, 3).reshape(B, Sq, Hq * Dh) @ wo

    def _B_ref(x, w1, b1, w2, b2):
        h = jnp.einsum("bsd,df->bsf", x, w1) + b1
        zero = jnp.zeros_like(h)
        r = jnp.where(h > zero, h, zero)
        h = r * r
        out = jnp.einsum("bsf,fd->bsd", h, w2) + b2
        return out

    x = A_x
    g = _sigmoid((x * gate_w).sum(-1, keepdims=True))
    a = _A_ref(x, A_k_cache, A_v_cache, A_wq, A_wo)
    b = _B_ref(x, B_w1, B_b1, B_w2, B_b2)
    return g * a + (1 - g) * b
```

```python
import functools

import jax
import jax.numpy as jnp
import jax.experimental.pallas as pl
import jax.experimental.pallas.tpu as pltpu

_F32 = jnp.float32
_BF16 = jnp.bfloat16


def _fused_kernel(x_ref, k_ref, v_ref, wq_ref, wo_ref, w1_ref, b1_ref, w2_ref,
                  b2_ref, gw_ref, o_ref, q_scr, ob_scr, acc_scr, mlp_scr,
                  *, n_b, rep, dh, scale):
    h = pl.program_id(0)
    b = pl.program_id(1)
    n_h = pl.num_programs(0)

    @pl.when(jnp.logical_and(h == 0, b == 0))
    def _():
        x = x_ref[...]
        hid = jnp.dot(x, w1_ref[...], preferred_element_type=_F32)
        hid = hid + b1_ref[...].astype(_F32)
        r = jnp.where(hid > 0.0, hid, 0.0)
        act = (r * r).astype(_BF16)
        mlp = jnp.dot(act, w2_ref[...], preferred_element_type=_F32)
        mlp_scr[...] = mlp + b2_ref[...].astype(_F32)
        acc_scr[...] = jnp.zeros_like(acc_scr)

    @pl.when(b == 0)
    def _():
        y = jnp.dot(x_ref[...], wq_ref[...], preferred_element_type=_F32)
        y = y.astype(_BF16).astype(_F32)
        for bb in range(n_b):
            for g in range(rep):
                q_scr[bb, g:g + 1, :] = y[bb:bb + 1, g * dh:(g + 1) * dh]

    q = q_scr[b].astype(_BF16)
    k = k_ref[0, 0]
    v = v_ref[0, 0]
    s = jax.lax.dot_general(q, k, (((1,), (1,)), ((), ())),
                            preferred_element_type=_F32) * scale
    m = jnp.max(s, axis=-1, keepdims=True)
    p = jnp.exp(s - m)
    l = jnp.sum(p, axis=-1, keepdims=True)
    o = jnp.dot(p.astype(_BF16), v, preferred_element_type=_F32) / l
    row = jax.lax.broadcasted_iota(jnp.int32, (n_b, dh), 0)
    for g in range(rep):
        old = jnp.where(b == 0, 0.0, ob_scr[:, g * dh:(g + 1) * dh])
        ob_scr[:, g * dh:(g + 1) * dh] = jnp.where(
            row == b, jnp.broadcast_to(o[g:g + 1, :], (n_b, dh)), old)

    @pl.when(b == n_b - 1)
    def _():
        acc_scr[...] += jnp.dot(ob_scr[...].astype(_BF16), wo_ref[...],
                                preferred_element_type=_F32)

    @pl.when(jnp.logical_and(h == n_h - 1, b == n_b - 1))
    def _():
        xg = x_ref[...].astype(_F32) * gw_ref[...].astype(_F32)
        g = jax.nn.sigmoid(jnp.sum(xg, axis=-1, keepdims=True))
        out = g * acc_scr[...] + (1.0 - g) * mlp_scr[...]
        o_ref[...] = out.astype(o_ref.dtype)


@jax.jit
def pallas_gated_mix__gqa_block_cached__dense_activation_squared_relu__decode_kernel(
    A_x: jax.Array,
    A_k_cache: jax.Array,
    A_v_cache: jax.Array,
    A_wq: jax.Array,
    A_wo: jax.Array,
    B_x: jax.Array,
    B_w1: jax.Array,
    B_b1: jax.Array,
    B_w2: jax.Array,
    B_b2: jax.Array,
    gate_w: jax.Array,
):
    del B_x
    n_b, sq, d = A_x.shape
    _, n_h, sk, dh = A_k_cache.shape
    hq = 32
    rep = hq // n_h
    f = B_w1.shape[1]
    gw = rep * dh
    scale = float(dh) ** -0.5

    x2 = A_x.reshape(n_b * sq, d)
    b1 = B_b1.reshape(1, f)
    b2 = B_b2.reshape(1, d)
    gwv = gate_w.reshape(1, d)

    kernel = functools.partial(_fused_kernel, n_b=n_b, rep=rep, dh=dh, scale=scale)

    out = pl.pallas_call(
        kernel,
        out_shape=jax.ShapeDtypeStruct((n_b * sq, d), A_x.dtype),
        grid=(n_h, n_b),
        in_specs=[
            pl.BlockSpec((n_b * sq, d), lambda h, b: (0, 0)),
            pl.BlockSpec((1, 1, sk, dh), lambda h, b: (b, h, 0, 0)),
            pl.BlockSpec((1, 1, sk, dh), lambda h, b: (b, h, 0, 0)),
            pl.BlockSpec((d, gw), lambda h, b: (0, h)),
            pl.BlockSpec((gw, d), lambda h, b: (h, 0)),
            pl.BlockSpec((d, f), lambda h, b: (0, 0)),
            pl.BlockSpec((1, f), lambda h, b: (0, 0)),
            pl.BlockSpec((f, d), lambda h, b: (0, 0)),
            pl.BlockSpec((1, d), lambda h, b: (0, 0)),
            pl.BlockSpec((1, d), lambda h, b: (0, 0)),
        ],
        out_specs=pl.BlockSpec((n_b * sq, d), lambda h, b: (0, 0)),
        scratch_shapes=[
            pltpu.VMEM((n_b, rep, dh), _F32),
            pltpu.VMEM((n_b, gw), _F32),
            pltpu.VMEM((n_b, d), _F32),
            pltpu.VMEM((n_b, d), _F32),
        ],
        compiler_params=pltpu.CompilerParams(
            dimension_semantics=("arbitrary", "arbitrary"),
            vmem_limit_bytes=64 * 1024 * 1024,
        ),
    )(x2, A_k_cache, A_v_cache, A_wq, A_wo, B_w1, b1, B_w2, b2, gwv)
    return out.reshape(n_b, sq, d)
```

```python
import functools

import jax
import jax.numpy as jnp
import jax.experimental.pallas as pl
import jax.experimental.pallas.tpu as pltpu

_F32 = jnp.float32
_BF16 = jnp.bfloat16


def _fused_kernel(x_ref, k_ref, v_ref, wq_ref, wo_ref, w1_ref, b1_ref, w2_ref,
                  b2_ref, gw_ref, o_ref, q_scr, ob_scr, acc_scr, mlp_scr,
                  *, n_b, rep, dh, scale):
    h = pl.program_id(0)
    b = pl.program_id(1)
    n_h = pl.num_programs(0)

    @pl.when(jnp.logical_and(h == 0, b == 0))
    def _():
        acc_scr[...] = jnp.zeros_like(acc_scr)

    @pl.when(jnp.logical_and(h == 0, b == 1))
    def _():
        x = x_ref[0]
        hid = jnp.dot(x, w1_ref[...], preferred_element_type=_F32)
        hid = hid + b1_ref[...].astype(_F32)
        r = jnp.where(hid > 0.0, hid, 0.0)
        act = (r * r).astype(_BF16)
        mlp = jnp.dot(act, w2_ref[...], preferred_element_type=_F32)
        mlp_scr[...] = mlp + b2_ref[...].astype(_F32)

    @pl.when(b == 0)
    def _():
        y = jnp.dot(x_ref[0], wq_ref[...], preferred_element_type=_F32)
        y = y.astype(_BF16).astype(_F32)
        for bb in range(n_b):
            for g in range(rep):
                q_scr[bb, g:g + 1, :] = y[bb:bb + 1, g * dh:(g + 1) * dh]

    q = q_scr[b].astype(_BF16)
    k = k_ref[0, 0]
    v = v_ref[0, 0]
    s = jax.lax.dot_general(q, k, (((1,), (1,)), ((), ())),
                            preferred_element_type=_F32) * scale
    m = jnp.max(s, axis=-1, keepdims=True)
    p = jnp.exp(s - m)
    l = jnp.sum(p, axis=-1, keepdims=True)
    o = jnp.dot(p.astype(_BF16), v, preferred_element_type=_F32) / l
    row = jax.lax.broadcasted_iota(jnp.int32, (n_b, dh), 0)
    for g in range(rep):
        old = jnp.where(b == 0, 0.0, ob_scr[:, g * dh:(g + 1) * dh])
        ob_scr[:, g * dh:(g + 1) * dh] = jnp.where(
            row == b, jnp.broadcast_to(o[g:g + 1, :], (n_b, dh)), old)

    @pl.when(b == n_b - 1)
    def _():
        acc_scr[...] += jnp.dot(ob_scr[...].astype(_BF16), wo_ref[...],
                                preferred_element_type=_F32)

    @pl.when(jnp.logical_and(h == n_h - 1, b == n_b - 1))
    def _():
        xg = x_ref[0].astype(_F32) * gw_ref[...].astype(_F32)
        g = jax.nn.sigmoid(jnp.sum(xg, axis=-1, keepdims=True))
        out = g * acc_scr[...] + (1.0 - g) * mlp_scr[...]
        o_ref[0] = out.astype(o_ref.dtype)


@jax.jit
def pallas_gated_mix__gqa_block_cached__dense_activation_squared_relu__decode_kernel(
    A_x: jax.Array,
    A_k_cache: jax.Array,
    A_v_cache: jax.Array,
    A_wq: jax.Array,
    A_wo: jax.Array,
    B_x: jax.Array,
    B_w1: jax.Array,
    B_b1: jax.Array,
    B_w2: jax.Array,
    B_b2: jax.Array,
    gate_w: jax.Array,
):
    del B_x
    n_b, sq, d = A_x.shape
    _, n_h, sk, dh = A_k_cache.shape
    hq = 32
    rep = hq // n_h
    f = B_w1.shape[1]
    gw = rep * dh
    scale = float(dh) ** -0.5


    kernel = functools.partial(_fused_kernel, n_b=n_b, rep=rep, dh=dh, scale=scale)

    out = pl.pallas_call(
        kernel,
        out_shape=jax.ShapeDtypeStruct((sq, n_b, d), A_x.dtype),
        grid=(n_h, n_b),
        in_specs=[
            pl.BlockSpec((sq, n_b, d), lambda h, b: (0, 0, 0)),
            pl.BlockSpec((1, 1, sk, dh), lambda h, b: (b, h, 0, 0)),
            pl.BlockSpec((1, 1, sk, dh), lambda h, b: (b, h, 0, 0)),
            pl.BlockSpec((d, gw), lambda h, b: (0, h)),
            pl.BlockSpec((gw, d), lambda h, b: (h, 0)),
            pl.BlockSpec((d, f), lambda h, b: (0, 0)),
            pl.BlockSpec((f,), lambda h, b: (0,)),
            pl.BlockSpec((f, d), lambda h, b: (0, 0)),
            pl.BlockSpec((d,), lambda h, b: (0,)),
            pl.BlockSpec((d,), lambda h, b: (0,)),
        ],
        out_specs=pl.BlockSpec((sq, n_b, d), lambda h, b: (0, 0, 0)),
        scratch_shapes=[
            pltpu.VMEM((n_b, rep, dh), _F32),
            pltpu.VMEM((n_b, gw), _F32),
            pltpu.VMEM((n_b, d), _F32),
            pltpu.VMEM((n_b, d), _F32),
        ],
        compiler_params=pltpu.CompilerParams(
            dimension_semantics=("arbitrary", "arbitrary"),
            vmem_limit_bytes=64 * 1024 * 1024,
        ),
    )(jnp.transpose(A_x, (1, 0, 2)), A_k_cache, A_v_cache, A_wq, A_wo, B_w1, B_b1, B_w2, B_b2, gate_w)
    return jnp.transpose(out, (1, 0, 2))
```

```python
import functools

import jax
import jax.numpy as jnp
import jax.experimental.pallas as pl
import jax.experimental.pallas.tpu as pltpu

_F32 = jnp.float32
_BF16 = jnp.bfloat16


def _fused_kernel(x_ref, k_ref, v_ref, k_hbm, v_hbm, wq_ref, wo_ref, w1_ref,
                  b1_ref, w2_ref, b2_ref, gw_ref, o_ref,
                  k_last, v_last, sems, q_scr, ob_scr, acc_scr, mlp_scr, g_scr,
                  *, n_b, n_blk, rep, dh, scale):
    t = pl.program_id(0)
    b = jax.lax.rem(t, n_b)
    last = n_blk - 1

    k_copy = pltpu.make_async_copy(k_hbm.at[last % n_b, last // n_b], k_last,
                                   sems.at[0])
    v_copy = pltpu.make_async_copy(v_hbm.at[last % n_b, last // n_b], v_last,
                                   sems.at[1])

    @pl.when(t == last - 2)
    def _():
        k_copy.start()
        v_copy.start()

    @pl.when(t == 0)
    def _():
        acc_scr[...] = jnp.zeros_like(acc_scr)

    @pl.when(t == 1)
    def _():
        x = x_ref[0]
        hid = jnp.dot(x, w1_ref[...], preferred_element_type=_F32)
        hid = hid + b1_ref[...].astype(_F32)
        r = jnp.where(hid > 0.0, hid, 0.0)
        mlp = jnp.dot((r * r).astype(_BF16), w2_ref[...],
                      preferred_element_type=_F32)
        mlp = mlp + b2_ref[...].astype(_F32)
        xg = x.astype(_F32) * gw_ref[...].astype(_F32)
        gate = jax.nn.sigmoid(jnp.sum(xg, axis=-1, keepdims=True))
        g_scr[...] = gate
        mlp_scr[...] = (1.0 - gate) * mlp

    @pl.when(b == 0)
    def _():
        y = jnp.dot(x_ref[0], wq_ref[...], preferred_element_type=_F32)
        y = y.astype(_BF16).astype(_F32)
        for bb in range(n_b):
            for g in range(rep):
                q_scr[bb, g:g + 1, :] = y[bb:bb + 1, g * dh:(g + 1) * dh]

    def attend(get_k, get_v):
        q = q_scr[b].astype(_BF16)
        s = jax.lax.dot_general(q, get_k(), (((1,), (1,)), ((), ())),
                                preferred_element_type=_F32) * scale
        m = jnp.max(s, axis=-1, keepdims=True)
        p = jnp.exp(s - m)
        l = jnp.sum(p, axis=-1, keepdims=True)
        o = jnp.dot(p.astype(_BF16), get_v(), preferred_element_type=_F32) / l
        row = jax.lax.broadcasted_iota(jnp.int32, (n_b, dh), 0)
        for g in range(rep):
            old = jnp.where(b == 0, 0.0, ob_scr[:, g * dh:(g + 1) * dh])
            ob_scr[:, g * dh:(g + 1) * dh] = jnp.where(
                row == b, jnp.broadcast_to(o[g:g + 1, :], (n_b, dh)), old)

    @pl.when(t < last)
    def _():
        attend(lambda: k_ref[0, 0], lambda: v_ref[0, 0])

    @pl.when(t == last)
    def _():
        def get_k():
            k_copy.wait()
            return k_last[...]

        def get_v():
            v_copy.wait()
            return v_last[...]

        attend(get_k, get_v)

    @pl.when(b == n_b - 1)
    def _():
        acc_scr[...] += jnp.dot(ob_scr[...].astype(_BF16), wo_ref[...],
                                preferred_element_type=_F32)

    @pl.when(t == last)
    def _():
        out = g_scr[...] * acc_scr[...] + mlp_scr[...]
        o_ref[0] = out.astype(o_ref.dtype)


@jax.jit
def pallas_gated_mix__gqa_block_cached__dense_activation_squared_relu__decode_kernel(
    A_x: jax.Array,
    A_k_cache: jax.Array,
    A_v_cache: jax.Array,
    A_wq: jax.Array,
    A_wo: jax.Array,
    B_x: jax.Array,
    B_w1: jax.Array,
    B_b1: jax.Array,
    B_w2: jax.Array,
    B_b2: jax.Array,
    gate_w: jax.Array,
):
    del B_x
    n_b, sq, d = A_x.shape
    _, n_h, sk, dh = A_k_cache.shape
    hq = 32
    rep = hq // n_h
    f = B_w1.shape[1]
    gw = rep * dh
    n_blk = n_h * n_b
    scale = float(dh) ** -0.5

    kernel = functools.partial(_fused_kernel, n_b=n_b, n_blk=n_blk, rep=rep,
                               dh=dh, scale=scale)

    def kv_map(t):
        tt = jnp.minimum(t, n_blk - 2)
        return (tt % n_b, tt // n_b, 0, 0)

    out = pl.pallas_call(
        kernel,
        out_shape=jax.ShapeDtypeStruct((sq, n_b, d), A_x.dtype),
        grid=(n_blk,),
        in_specs=[
            pl.BlockSpec((sq, n_b, d), lambda t: (0, 0, 0)),
            pl.BlockSpec((1, 1, sk, dh), kv_map),
            pl.BlockSpec((1, 1, sk, dh), kv_map),
            pl.BlockSpec(memory_space=pl.ANY),
            pl.BlockSpec(memory_space=pl.ANY),
            pl.BlockSpec((d, gw), lambda t: (0, t // n_b)),
            pl.BlockSpec((gw, d), lambda t: (t // n_b, 0)),
            pl.BlockSpec((d, f), lambda t: (0, 0)),
            pl.BlockSpec((f,), lambda t: (0,)),
            pl.BlockSpec((f, d), lambda t: (0, 0)),
            pl.BlockSpec((d,), lambda t: (0,)),
            pl.BlockSpec((d,), lambda t: (0,)),
        ],
        out_specs=pl.BlockSpec((sq, n_b, d), lambda t: (0, 0, 0)),
        scratch_shapes=[
            pltpu.VMEM((sk, dh), A_k_cache.dtype),
            pltpu.VMEM((sk, dh), A_v_cache.dtype),
            pltpu.SemaphoreType.DMA((2,)),
            pltpu.VMEM((n_b, rep, dh), _F32),
            pltpu.VMEM((n_b, gw), _F32),
            pltpu.VMEM((n_b, d), _F32),
            pltpu.VMEM((n_b, d), _F32),
            pltpu.VMEM((n_b, 1), _F32),
        ],
        compiler_params=pltpu.CompilerParams(
            dimension_semantics=("arbitrary",),
            vmem_limit_bytes=64 * 1024 * 1024,
        ),
    )(jnp.transpose(A_x, (1, 0, 2)), A_k_cache, A_v_cache, A_k_cache, A_v_cache,
      A_wq, A_wo, B_w1, B_b1, B_w2, B_b2, gate_w)
    return jnp.transpose(out, (1, 0, 2))
```
